```python
import os as _os
_os.environ.setdefault("JAX_PLATFORMS", "cpu")
import jax
import jax.numpy as jnp

def _softmax(x, axis=-1):
    return jax.nn.softmax(x, axis=axis)
def _gelu(x):
    return jax.nn.gelu(x, approximate=True)
def _silu(x):
    return jax.nn.silu(x)
def _sigmoid(x):
    return jax.nn.sigmoid(x)
def _layernorm(x, axis=-1, eps=1e-5):
    m = jnp.mean(x, axis=axis, keepdims=True)
    v = jnp.var(x, axis=axis, keepdims=True)
    return (x - m) / jnp.sqrt(v + eps)
def _scatter_add(tgt, idx, src, axis=0):
    return tgt.at[idx].add(src)
def _segment_sum(src, seg, n):
    return jax.ops.segment_sum(src, seg, n)
class _Rng:
    def __init__(self, key):
        self._k = key
    def _next(self):
        self._k, sub = jax.random.split(self._k)
        return sub
    def normal(self, shape):
        return jax.random.normal(self._next(), shape, dtype=jnp.bfloat16)
    def randint(self, lo, hi, shape):
        return jax.random.randint(self._next(), shape, lo, hi, dtype=jnp.int32)
    def uniform(self, shape, lo=0.0, hi=1.0):
        return jax.random.uniform(self._next(), shape, jnp.bfloat16, lo, hi)
    def permutation(self, n):
        return jax.random.permutation(self._next(), n)


kernel_name = 'standalone__batchnorm__sampling'

def setup_inputs():
    _rng = _Rng(jax.random.key(int.from_bytes(__import__("os").urandom(4), "little")))
    _w = (lambda a: (lambda t: t.astype(jnp.bfloat16) if jnp.issubdtype(t.dtype, jnp.floating) else t)(jnp.asarray(a)))
    B, S, C = 1024, 8, 640
    K = 3
    return {
        "x": _w((lambda *s: _rng.normal(s) * 0.05)(B, S, C)),
        "w": _w((lambda *s: _rng.normal(s) * 0.05)(K, C, C) * (1.0 / (K * C) ** 0.5)),
        "mean": _w((lambda *s: _rng.normal(s) * 0.05)(C) * 0.1),
        "var": _w(jnp.abs((lambda *s: _rng.normal(s) * 0.05)(C)) + 0.5),
        "g": _w((lambda *s: _rng.normal(s) * 0.05)(C) + 1.0),
        "b": _w((lambda *s: _rng.normal(s) * 0.05)(C) * 0.1),
    }

def reference(x, w, mean, var, g, b):
    K = 3
    P = K // 2
    S = x.shape[1]
    xp = jnp.pad(x, ((0, 0), (P, P), (0, 0)))
    y = sum(jnp.einsum('bsc,cd->bsd', xp[:, k:k + S, :], w[k]) for k in range(K))
    inv_std = 1.0 / jnp.sqrt(var + 1e-5)
    y = (y - mean) * (g * inv_std) + b
    return _silu(y)
```

```python
import contextlib
import functools
import jax
import jax.numpy as jnp
import jax.experimental.pallas as pl
import jax.experimental.pallas.tpu as pltpu

A = 0.625
Bp = 1.6
A2, B2 = A * A, Bp * Bp
A3, B3 = A2 * A, B2 * Bp
CC = A2 + B2
NA = 2 * A2 * (A2 - B2)
NB = 2 * B2 * (B2 - A2)
F32 = jnp.float32
BF16 = jnp.bfloat16
U32 = jnp.uint32
S = 8
RB = 16


def _in_transform(d0, d1, d2, d3, d4, d5):
    t_b2 = B2 * d2
    t_a2 = A2 * d2
    e1 = d4 - t_b2
    e2 = d4 - t_a2
    o1 = A * d3 - (A * B2) * d1
    o2 = Bp * d3 - (Bp * A2) * d1
    v0 = e1 - t_a2
    if d0 is not None:
        v0 = v0 + d0
    v5 = d1 - CC * d3
    if d5 is not None:
        v5 = v5 + d5
    return [v0, e1 + o1, e1 - o1, e2 + o2, e2 - o2, v5]


def _rep(v, k):
    return v if k == 1 else jnp.concatenate([v] * k, axis=0)


def _t_store(xs, v_ref, c, rb, nb):
    v_t0 = _in_transform(None, xs[0], xs[1], xs[2], xs[3], xs[4])
    v_t1 = _in_transform(xs[3], xs[4], xs[5], xs[6], xs[7], None)
    for j in range(6):
        v_ref[j, c, pl.ds(rb * RB, RB), :] = v_t0[j].astype(BF16)
        v_ref[j, c, pl.ds(nb + rb * RB, RB), :] = v_t1[j].astype(BF16)


def _t_group(xu, v_ref, c, b0, rb, nb, NC, gate=None):
    if gate is None:
        sh = jnp.uint32(16)
        mk = jnp.uint32(0xFFFF0000)
    else:
        sh = _rep(gate | jnp.uint32(16), RB // 8)
        mk = _rep(gate | jnp.uint32(0xFFFF0000), RB // 8)
    xs = []
    for p in range(4):
        wd = xu[pl.ds((b0 + rb * RB) * 4 * NC + c * 4 + p, RB, stride=4 * NC), :]
        xs.append(pltpu.bitcast(wd << sh, F32))
        xs.append(pltpu.bitcast(wd & mk, F32))
    _t_store(xs, v_ref, c, rb, nb)


def _t0_group(xk, st, v_ref, c, rb, nb, gate=None):
    r0 = (c * (nb // RB) + rb) * RB * S
    u = pltpu.bitcast(xk[pl.ds(rb * RB, RB), pl.ds(c * S, S), :].reshape(RB * S, 128), U32)
    if gate is not None:
        u = u | _rep(gate, RB * S // 16)
    st[pl.ds(r0 // 2, RB * S // 2), :] = u
    xs = []
    for p in range(4):
        wd = st[pl.ds(r0 // 2 + p, RB, stride=4), :]
        xs.append(pltpu.bitcast(wd << 16, F32))
        xs.append(pltpu.bitcast(wd & jnp.uint32(0xFFFF0000), F32))
    _t_store(xs, v_ref, c, rb, nb)


def _wt_piece(gw, wl, n, r0, WR):
    rs = pl.ds(r0, WR)
    ns = pl.ds(n * 128, 128)
    gwu = gw.bitcast(U32)
    rh = pl.ds(r0 // 2, WR // 2)
    u0, u1, u2 = [pltpu.bitcast(wl[k, rs, ns], U32) for k in range(3)]
    gwu[0, n, rh, :] = u0
    gwu[5, n, rh, :] = u2
    g0, g1, g2 = [pltpu.bitcast(u, BF16).astype(F32) for u in (u0, u1, u2)]
    ea = g0 * (1.0 / NA) + g2 * (A2 / NA)
    oa = g1 * (A / NA)
    gw[1, n, rs, :] = (ea + oa).astype(BF16)
    gw[2, n, rs, :] = (ea - oa).astype(BF16)
    eb = g0 * (1.0 / NB) + g2 * (B2 / NB)
    ob = g1 * (Bp / NB)
    gw[3, n, rs, :] = (eb + ob).astype(BF16)
    gw[4, n, rs, :] = (eb - ob).astype(BF16)


def _epilogue(ms, ou, ss, n, b0, nb, NC, tiles=(0, 1)):
    ns = slice(n * 128, (n + 1) * 128)
    cf = [ss[k:k + 1, ns] for k in range(8)]
    sc, sh = cf[0], cf[1]
    s1 = ms[1] + ms[2]
    d1 = ms[1] - ms[2]
    s2 = ms[3] + ms[4]
    d2 = ms[3] - ms[4]
    h = [
        (ms[0] + s1 + s2) * sc + sh,
        d1 * cf[2] + d2 * cf[3] + sh,
        s1 * cf[4] + s2 * cf[5] + sh,
        d1 * cf[6] + d2 * cf[7] + ms[5] * sc + sh,
    ]
    z = [hh + hh * jnp.tanh(hh) for hh in h]
    zr = [pltpu.bitcast(zz.astype(BF16).astype(F32), U32) for zz in z]
    p01 = (zr[0] >> 16) | zr[1]
    p23 = (zr[2] >> 16) | zr[3]
    base = b0 * 4 * NC + n * 4
    for k, t in enumerate(tiles):
        ou[pl.ds(base + 2 * t, nb, stride=4 * NC), :] = p01[k * nb:(k + 1) * nb]
        ou[pl.ds(base + 2 * t + 1, nb, stride=4 * NC), :] = p23[k * nb:(k + 1) * nb]


def _epi_dyn(m_ref, ou0, ss, n, t, rq, r0, ne, nb, NC, gate=None):
    ms = [m_ref[n, j, pl.ds(pl.multiple_of(rq + (t * nb + r0), 8), ne), :] for j in range(6)]
    if gate is not None:
        gt = _rep(gate, ne // 8)
        for j in (0, 1, 3, 5):
            ms[j] = pltpu.bitcast(pltpu.bitcast(ms[j], U32) | gt, F32)
    _epilogue(ms, ou0, ss, n, r0, ne, NC, tiles=(t,))


def _make_sched(plan, nvr):
    sched = {}
    for tasks, dots in plan:
        total = len(dots) * nvr
        for k, t in enumerate(tasks):
            pos = (k * total) // len(tasks)
            sched.setdefault(dots[pos // nvr], []).append((pos % nvr, t))
    return sched


def _mm_region(v_cur, gw, zero, NC, nb, plan, sink, split_last, r0=0, nr=None):
    nr = nb if nr is None else nr
    vcu = v_cur.bitcast(U32)
    gwu = gw.bitcast(U32)
    sched = _make_sched(plan, 2 * nr // 8)
    ndots = NC * 6
    d = 0
    for n in range(NC):
        ms = []
        for j in range(6):
            rhs = pltpu.bitcast(gwu[j, n], BF16)

            def lhs_of(a, b):
                return jnp.concatenate(
                    [pltpu.bitcast(vcu[j, c, pl.ds(a, b - a), :], BF16) for c in range(NC)], axis=1)
            t0 = (r0 // 2, (r0 + nr) // 2)
            t1 = ((nb + r0) // 2, (nb + r0 + nr) // 2)
            if split_last and d == ndots - 1:
                m = jnp.concatenate([jnp.dot(lhs_of(*t0), rhs, preferred_element_type=F32),
                                     jnp.dot(lhs_of(*t1), rhs, preferred_element_type=F32)], axis=0)
            elif nr == nb:
                m = jnp.dot(lhs_of(0, nb), rhs, preferred_element_type=F32)
            else:
                m = jnp.dot(jnp.concatenate([lhs_of(*t0), lhs_of(*t1)], axis=0), rhs,
                            preferred_element_type=F32)
            ms.append(m)
            for r, t in sched.get(d, []):
                t(pltpu.bitcast(m[r * 8:(r + 1) * 8, :], U32) & zero)
            d += 1
        sink(n, ms)


def _k_region(v_cur, gw, ma, zero, NC, nb, cs, first, plan, jorder, nsplit, rsubs, pre):
    vcu = v_cur.bitcast(U32)
    gwu = gw.bitcast(U32)
    nvr = 2 * min(rsubs) // 8
    sched = _make_sched(plan, nvr)
    ndots = NC * 6 * len(rsubs)
    rh = pl.ds(cs[0] * 64, len(cs) * 64)
    d = 0
    b0 = 0
    for k, nr in enumerate(rsubs):
        for t in pre[k]:
            t()
        order = ([(j, n) for j in jorder for n in range(NC)] if first
                 else [(j, n) for n in range(NC) for j in jorder])
        for j, n in order:
            if True:
                rhs = pltpu.bitcast(gwu[j, n, rh, :], BF16)

                def lhs_of(a, b):
                    return jnp.concatenate(
                        [pltpu.bitcast(vcu[j, c, pl.ds(a // 2, (b - a) // 2), :], BF16) for c in cs], axis=1)

                def fin(m, ranges):
                    off = 0
                    outs = []
                    for a, b in ranges:
                        mm = m[off:off + (b - a)]
                        if not first:
                            mm = mm + ma[n, j, pl.ds(a, b - a), :]
                        ma[n, j, pl.ds(a, b - a), :] = mm
                        outs.append(mm)
                        off += b - a
                    return outs[0] if len(outs) == 1 else jnp.concatenate(outs, axis=0)
                t0 = (b0, b0 + nr)
                t1 = (nb + b0, nb + b0 + nr)
                if d >= ndots - nsplit:
                    m = jnp.concatenate([fin(jnp.dot(lhs_of(*t0), rhs, preferred_element_type=F32), [t0]),
                                         fin(jnp.dot(lhs_of(*t1), rhs, preferred_element_type=F32), [t1])], axis=0)
                elif nr == nb:
                    m = fin(jnp.dot(lhs_of(0, 2 * nb), rhs, preferred_element_type=F32), [(0, 2 * nb)])
                else:
                    m = fin(jnp.dot(jnp.concatenate([lhs_of(*t0), lhs_of(*t1)], axis=0), rhs,
                                    preferred_element_type=F32), [t0, t1])
                for r, t in sched.get(d, []):
                    t(pltpu.bitcast(m[r * 8:(r + 1) * 8, :], U32) & zero)
                d += 1
        b0 += nr


def _kernel(x3_hbm, x_hbm, w_hbm, mean_hbm, var_hbm, g_hbm, b_hbm, o_hbm,
            xk, st, xall, oall, o0, va, vb, ma, gw, wl, pm, pv, pg, pb, ss,
            x0sem, xsem, osem, lsem, o0sem, wsem, psem, *, NB0, SB, NSUB, LAST, WR, KG, SCOPES, EB,
            GJ, GEND, TD, EDOTS, JO, XQ0, NSPL, RS, T0D):
    C = w_hbm.shape[-1]
    B = x3_hbm.shape[0]
    NC = C // 128
    rpb = S * NC
    q = pl.program_id(0)
    nq = pl.num_programs(0)
    zero = jnp.full((8, 128), jax.lax.shift_right_logical(q, 24), jnp.int32).astype(U32)
    PB = SB * NSUB
    NL = sum(LAST)
    NQ = (B - NB0 - NL) // PB
    REST = NL - SB
    xu_all = xall.bitcast(U32)
    ou_all = oall.bitcast(U32)

    def scope(name):
        return jax.named_scope(name) if SCOPES else contextlib.nullcontext()

    def cp_in(b0, nb, sem):
        sl = pl.ds(b0 * rpb, nb * rpb)
        return pltpu.make_async_copy(x_hbm.at[sl, :], xall.at[sl, :], sem)

    def cp_out(b0, nb, sem):
        sl = pl.ds(b0 * rpb, nb * rpb)
        return pltpu.make_async_copy(oall.at[sl, :], o_hbm.at[sl, :], sem)

    RQ = -(-NB0 // (NQ * EB)) * EB
    rqs = [min(k * RQ, NB0 - RQ) for k in range(NQ)] + [NB0]

    def o0_copy(k):
        sl = pl.ds(rqs[k] * rpb, (rqs[k + 1] - rqs[k]) * rpb)
        return pltpu.make_async_copy(o0.at[sl, :], o_hbm.at[sl, :], o0sem.at[k])

    def xk_copy(gi):
        cs = KG[gi]
        sl = pl.ds(cs[0] * S, len(cs) * S)
        return pltpu.make_async_copy(x3_hbm.at[pl.ds(0, NB0), sl, :], xk.at[:, sl, :], x0sem.at[gi])

    def wk_copy(gi):
        cs = KG[gi]
        sl = pl.ds(cs[0] * 128, len(cs) * 128)
        return pltpu.make_async_copy(w_hbm.at[:, sl, :], wl.at[:, sl, :], wsem.at[gi])

    def x1_copy():
        return cp_in(NB0, SB, x0sem.at[len(KG)])

    def xq_copy(k, static_last=False):
        if static_last:
            return cp_in(NB0 + SB + NQ * PB, REST, xsem.at[NQ])
        return cp_in(pl.multiple_of(NB0 + SB + k * PB, 16), PB, xsem.at[k])

    def p_copies():
        return [pltpu.make_async_copy(s, d, psem.at[k])
                for k, (s, d) in enumerate(((mean_hbm, pm), (var_hbm, pv), (g_hbm, pg), (b_hbm, pb)))]

    def t_tasks(xu, v_ref, b0, nb):
        return [functools.partial(_t_group, xu, v_ref, c, b0, rb, nb, NC)
                for c in range(NC) for rb in range(nb // RB)]

    gdots = [d for d in range(6 * NC - GEND) if d % 6 in GJ]

    @pl.when(q == 0)
    def _():
        for gi in range(len(KG)):
            pr = 0 if gi == 0 else 1
            xk_copy(gi).start(priority=pr)
            wk_copy(gi).start(priority=pr)
        x1_copy().start(priority=1)
        for cp in p_copies():
            cp.start(priority=1)
        for gi, cs in enumerate(KG):
            last = gi == len(KG) - 1
            if gi == 0:
                with scope("xw0"):
                    xk_copy(0).wait()
                with scope("T00"):
                    for c in cs:
                        for rb in range(NB0 // RB):
                            _t0_group(xk, st, va, c, rb, NB0)
            with scope(f"ww{gi}"):
                if gi > 0:
                    xk_copy(gi).wait()
                wk_copy(gi).wait()
                if gi == XQ0:
                    xq_copy(0).start(priority=1)
                if last:
                    x1_copy().wait()
                    for cp in p_copies():
                        cp.wait()
            with scope(f"R0_{gi}"):
                if last:
                    mean = pm[...].astype(F32).reshape(1, C)
                    var = pv[...].astype(F32).reshape(1, C)
                    g = pg[...].astype(F32).reshape(1, C)
                    b = pb[...].astype(F32).reshape(1, C)
                    scf = g * jax.lax.rsqrt(var + 1e-5)
                    sc = scf * 0.5
                    ss[0:1, :] = sc
                    ss[1:2, :] = (b - mean * scf) * 0.5
                    for k, cst in enumerate((A, Bp, A2, B2, A3, B3)):
                        ss[2 + k:3 + k, :] = sc * cst
                rsubs = RS[gi]
                pre = []
                plan = []
                b0 = 0
                for k, nr in enumerate(rsubs):
                    th = []
                    if gi > 0:
                        for rb in range(b0 // RB, (b0 + nr) // RB):
                            for c in cs:
                                th.append(functools.partial(_t0_group, xk, st, va, c, rb, NB0))
                    if k > 0 and th:
                        plan.append((th, [(k - 1) * 30 + d for d in T0D[min(k - 1, len(T0D) - 1)]]))
                        th = []
                    if k == 0:
                        for n in range(NC):
                            for r0 in range(cs[0] * 128, (cs[-1] + 1) * 128, WR):
                                th.append(functools.partial(_wt_piece, gw, wl, n, r0, WR))
                    pre.append(th)
                    b0 += nr
                if last:
                    plan.append((t_tasks(xu_all, vb, NB0, SB), list(TD)))
                _k_region(va, gw, ma, zero, NC, NB0, cs, gi == 0, plan, JO, NSPL, rsubs, pre)

    with scope("xw"):
        xq_copy(q).wait()
        for k in range(NQ - 1):
            @pl.when(q == k + 1)
            def _(k=k):
                o0_copy(k).start()

        @pl.when(q < nq - 1)
        def _():
            xq_copy(q + 1).start()

        if REST:
            @pl.when(q == nq - 1)
            def _():
                xq_copy(0, static_last=True).start()
    with scope("body"):
        base = pl.multiple_of(NB0 + q * PB, 16)
        xu = xall.at[pl.ds(base * rpb, (PB + SB) * rpb), :].bitcast(U32)
        ou = oall.at[pl.ds(base * rpb, PB * rpb), :].bitcast(U32)
        vbufs = (vb, va)
        rq = pl.multiple_of(jnp.minimum(q * RQ, NB0 - RQ), EB)
        ou0 = o0.at[pl.ds(rq * rpb, RQ * rpb), :].bitcast(U32)
        e0 = [functools.partial(_epi_dyn, ma, ou0, ss, n, t, rq, r0, EB, NB0, NC)
              for n in range(NC) for t in range(2) for r0 in range(0, RQ, EB)]
        for k in range(NSUB):
            ek = e0[(k * len(e0)) // NSUB:((k + 1) * len(e0)) // NSUB]
            _mm_region(vbufs[k % 2], gw, zero, NC, SB,
                       [(t_tasks(xu, vbufs[(k + 1) % 2], (k + 1) * SB, SB), gdots), (ek, EDOTS)],
                       lambda n, ms, k=k: _epilogue(ms, ou, ss, n, k * SB, SB, NC), k == NSUB - 1)
            cp_out(base + k * SB, SB, osem.at[q * NSUB + k]).start()

    @pl.when(q == nq - 1)
    def _():
        bl = NB0 + NQ * PB
        if REST:
            with scope("xwl"):
                xq_copy(0, static_last=True).wait()
        pieces = []
        pos = 0
        for nr in LAST:
            if pos < SB:
                assert pos + nr <= SB
                pieces.append((vb, SB, pos, nr))
            else:
                pieces.append((va, REST, pos - SB, nr))
            pos += nr
        with scope("L"):
            o0_copy(NQ - 1).start()
            pos = 0
            for k, (vr, nbk, r0, nr) in enumerate(pieces):
                plan = []
                if k == 0 and REST:
                    plan = [(t_tasks(xu_all, va, bl + SB, REST), gdots)]
                _mm_region(vr, gw, zero, NC, nbk, plan,
                           lambda n, ms, pos=pos, nr=nr: _epilogue(ms, ou_all, ss, n, bl + pos, nr, NC),
                           k == len(pieces) - 1, r0=r0, nr=nr)
                cp_out(bl + pos, nr, lsem.at[k]).start()
                pos += nr
        with scope("owait"):
            for k in range(NQ):
                o0_copy(k).wait()
            for k in range(NQ * NSUB):
                cp_out(NB0 + k * SB, SB, osem.at[k]).wait()
            pos = 0
            for k, nr in enumerate(LAST):
                cp_out(bl + pos, nr, lsem.at[k]).wait()
                pos += nr


def make(NB0=192, SB=64, NSUB=4, LAST=(32, 32), WR=32, KG=((0,), (1, 2), (3, 4)),
         SCOPES=False, EB=8, GJ=(1, 2, 3), GEND=3, TD=tuple(range(32, 57)),
         EDOTS=(2, 3, 4, 8, 9, 10, 14, 15, 16, 20, 21, 22, 26), JO=(0, 5, 1, 2, 3, 4), XQ0=1, NSPL=2, RS=((192,), (96, 96), (96, 96)), T0D=(tuple(range(4, 27)), tuple(range(0, 26)))):
    @jax.jit
    def f(x, w, mean, var, g, b):
        B, _, C = x.shape
        NC = C // 128
        PB = SB * NSUB
        NQ = (B - NB0 - sum(LAST)) // PB
        assert NB0 + NQ * PB + sum(LAST) == B and NSUB % 2 == 0 and sum(LAST) >= SB
        mb = max(NB0, SB, sum(LAST) - SB)
        x4 = x.reshape(B, S, NC, 128).transpose(0, 2, 1, 3)
        x2 = x4.reshape(B * NC * S, 128)
        x3 = x4.reshape(B, NC * S, 128)
        anyspec = pl.BlockSpec(memory_space=pl.ANY)
        out = pl.pallas_call(
            functools.partial(_kernel, NB0=NB0, SB=SB, NSUB=NSUB, LAST=LAST, WR=WR, KG=KG,
                              SCOPES=SCOPES, EB=EB, GJ=GJ, GEND=GEND, TD=TD, EDOTS=list(EDOTS), JO=JO,
                              XQ0=XQ0, NSPL=NSPL, RS=RS, T0D=T0D),
            grid=(NQ,),
            in_specs=[anyspec] * 7,
            out_specs=anyspec,
            out_shape=jax.ShapeDtypeStruct((B * S * NC, 128), x.dtype),
            scratch_shapes=[
                pltpu.VMEM((NB0, S * NC, 128), BF16),
                pltpu.VMEM((NB0 * S * NC // 2, 128), U32),
                pltpu.VMEM((B * S * NC, 128), BF16), pltpu.VMEM((B * S * NC, 128), BF16),
                pltpu.VMEM((NB0 * S * NC, 128), BF16),
                pltpu.VMEM((6, NC, 2 * mb, 128), BF16), pltpu.VMEM((6, NC, 2 * mb, 128), BF16),
                pltpu.VMEM((NC, 6, 2 * NB0, 128), F32),
                pltpu.VMEM((6, NC, C, 128), BF16),
                pltpu.VMEM((3, C, C), BF16),
                pltpu.VMEM((C,), BF16), pltpu.VMEM((C,), BF16),
                pltpu.VMEM((C,), BF16), pltpu.VMEM((C,), BF16),
                pltpu.VMEM((8, C), F32),
                pltpu.SemaphoreType.DMA((len(KG) + 1,)),
                pltpu.SemaphoreType.DMA((NQ + 1,)),
                pltpu.SemaphoreType.DMA((NQ * NSUB,)),
                pltpu.SemaphoreType.DMA((len(LAST),)),
                pltpu.SemaphoreType.DMA((NQ,)),
                pltpu.SemaphoreType.DMA((len(KG),)), pltpu.SemaphoreType.DMA((4,)),
            ],
            compiler_params=pltpu.CompilerParams(
                dimension_semantics=("arbitrary",),
                vmem_limit_bytes=100 * 1024 * 1024,
            ),
        )(x3, x2, w, mean, var, g, b)
        return out.reshape(B, NC, S, 128).transpose(0, 2, 1, 3).reshape(B, S, C)
    return f


_impl = make()


@jax.jit
def pallas_standalone__batchnorm__sampling_kernel(x, w, mean, var, g, b):
    return _impl(x, w, mean, var, g, b)
```

```python
import functools

import jax
import jax.numpy as jnp
import jax.experimental.pallas as pl
import jax.experimental.pallas.tpu as pltpu

F32 = jnp.float32
BF16 = jnp.bfloat16
U32 = jnp.uint32

PA = 0.625
PB_ = 1.6
A2, B2 = PA * PA, PB_ * PB_
A3, B3 = A2 * PA, B2 * PB_
CC = A2 + B2
NA = 2 * A2 * (A2 - B2)
NB = 2 * B2 * (B2 - A2)

S = 8
RB = 16
EB = 8
WR = 32

NB0 = 192
SB = 64
NSUB = 4
LAST = (32, 16, 16)
KG = ((0,), (1, 2), (3, 4))
R0P = (
    dict(wait=0, items=((0, 0, 192),)),
    dict(wait=1, t0pre=96, items=((1, 0, 96), (1, 96, 64)),
         t0x=((1, 192, tuple(range(32, 56))),)),
    dict(wait=2, items=((1, 160, 32), (2, 0, 96), (2, 96, 96))),
)
JO = (0, 5, 1, 2, 3, 4)
GDOTS = tuple(d for d in range(27) if d % 6 in (1, 2))
EDOTS = (3, 9, 15, 21, 27)
TD = tuple(range(60, 88))
T0D = tuple(range(0, 26))


def _in_transform(d0, d1, d2, d3, d4, d5):
    t_b2 = B2 * d2
    t_a2 = A2 * d2
    e1 = d4 - t_b2
    e2 = d4 - t_a2
    o1 = PA * d3 - (PA * B2) * d1
    o2 = PB_ * d3 - (PB_ * A2) * d1
    v0 = e1 - t_a2
    if d0 is not None:
        v0 = v0 + d0
    v5 = d1 - CC * d3
    if d5 is not None:
        v5 = v5 + d5
    return [v0, e1 + o1, e1 - o1, e2 + o2, e2 - o2, v5]


def _rep(v, k):
    return v if k == 1 else jnp.concatenate([v] * k, axis=0)


def _t_store(xs, v_ref, c, rb, nb):
    v_t0 = _in_transform(None, xs[0], xs[1], xs[2], xs[3], xs[4])
    v_t1 = _in_transform(xs[3], xs[4], xs[5], xs[6], xs[7], None)
    for j in range(6):
        v_ref[j, c, pl.ds(rb * RB, RB), :] = v_t0[j].astype(BF16)
        v_ref[j, c, pl.ds(nb + rb * RB, RB), :] = v_t1[j].astype(BF16)


def _t_group(xu, v_ref, c, b0, rb, nb, nc, gate):
    sh = _rep(gate | jnp.uint32(16), RB // 8)
    mk = _rep(gate | jnp.uint32(0xFFFF0000), RB // 8)
    xs = []
    for p in range(4):
        wd = xu[pl.ds((b0 + rb * RB) * 4 * nc + c * 4 + p, RB, stride=4 * nc), :]
        xs.append(pltpu.bitcast(wd << sh, F32))
        xs.append(pltpu.bitcast(wd & mk, F32))
    _t_store(xs, v_ref, c, rb, nb)


def _t0_group(xk, st, v_ref, c, rb, nb, gate=None):
    r0 = (c * (nb // RB) + rb) * RB * S // 2
    u = pltpu.bitcast(
        xk[pl.ds(rb * RB, RB), pl.ds(c * S, S), :].reshape(RB * S, 128), U32)
    if gate is not None:
        u = u | _rep(gate, RB * S // 16)
    st[pl.ds(r0, RB * S // 2), :] = u
    xs = []
    for p in range(4):
        wd = st[pl.ds(r0 + p, RB, stride=4), :]
        xs.append(pltpu.bitcast(wd << 16, F32))
        xs.append(pltpu.bitcast(wd & jnp.uint32(0xFFFF0000), F32))
    _t_store(xs, v_ref, c, rb, nb)


def _wt_piece(gw, wl, n, r0):
    rs = pl.ds(r0, WR)
    ns = pl.ds(n * 128, 128)
    gwu = gw.bitcast(U32)
    rh = pl.ds(r0 // 2, WR // 2)
    u0, u1, u2 = [pltpu.bitcast(wl[k, rs, ns], U32) for k in range(3)]
    gwu[0, n, rh, :] = u0
    gwu[5, n, rh, :] = u2
    g0, g1, g2 = [pltpu.bitcast(u, BF16).astype(F32) for u in (u0, u1, u2)]
    ea = g0 * (1.0 / NA) + g2 * (A2 / NA)
    oa = g1 * (PA / NA)
    gw[1, n, rs, :] = (ea + oa).astype(BF16)
    gw[2, n, rs, :] = (ea - oa).astype(BF16)
    eb = g0 * (1.0 / NB) + g2 * (B2 / NB)
    ob = g1 * (PB_ / NB)
    gw[3, n, rs, :] = (eb + ob).astype(BF16)
    gw[4, n, rs, :] = (eb - ob).astype(BF16)


def _epilogue(ms, ou, ss, n, b0, nb, nc, tiles=(0, 1)):
    ns = slice(n * 128, (n + 1) * 128)
    cf = [ss[k:k + 1, ns] for k in range(8)]
    sc, sh = cf[0], cf[1]
    s1 = ms[1] + ms[2]
    d1 = ms[1] - ms[2]
    s2 = ms[3] + ms[4]
    d2 = ms[3] - ms[4]
    h = [
        (ms[0] + s1 + s2) * sc + sh,
        d1 * cf[2] + d2 * cf[3] + sh,
        s1 * cf[4] + s2 * cf[5] + sh,
        d1 * cf[6] + d2 * cf[7] + ms[5] * sc + sh,
    ]
    z = [hh + hh * jnp.tanh(hh) for hh in h]
    zr = [pltpu.bitcast(zz.astype(BF16).astype(F32), U32) for zz in z]
    p01 = (zr[0] >> 16) | zr[1]
    p23 = (zr[2] >> 16) | zr[3]
    base = b0 * 4 * nc + n * 4
    for k, t in enumerate(tiles):
        ou[pl.ds(base + 2 * t, nb, stride=4 * nc), :] = p01[k * nb:(k + 1) * nb]
        ou[pl.ds(base + 2 * t + 1, nb, stride=4 * nc), :] = p23[k * nb:(k + 1) * nb]


def _epi_deferred(m_ref, ou0, ss, n, t, rq, r0, nc, gate):
    ms = [m_ref[n, j, pl.ds(pl.multiple_of(rq + (t * NB0 + r0), 8), EB), :]
          for j in range(6)]
    gt = _rep(gate, EB // 8)
    for j in (0, 1, 3, 5):
        ms[j] = pltpu.bitcast(pltpu.bitcast(ms[j], U32) | gt, F32)
    _epilogue(ms, ou0, ss, n, r0, EB, nc, tiles=(t,))


def _make_sched(plan, nvr):
    sched = {}
    for tasks, dots in plan:
        total = len(dots) * nvr
        for k, t in enumerate(tasks):
            pos = (k * total) // len(tasks)
            sched.setdefault(dots[pos // nvr], []).append((pos % nvr, t))
    return sched


def _dot(lhs, rhs):
    return jnp.dot(lhs, rhs, preferred_element_type=F32)


def _mm_region(v_cur, gw, zero, nc, nb, plan, sink, split_last, r0=0, nr=None):
    nr = nb if nr is None else nr
    vcu = v_cur.bitcast(U32)
    gwu = gw.bitcast(U32)
    sched = _make_sched(plan, 2 * nr // 8)
    t0 = (r0 // 2, (r0 + nr) // 2)
    t1 = ((nb + r0) // 2, (nb + r0 + nr) // 2)
    d = 0
    for n in range(nc):
        ms = []
        for j in range(6):
            rhs = pltpu.bitcast(gwu[j, n], BF16)

            def lhs_of(a, b, j=j):
                return jnp.concatenate(
                    [pltpu.bitcast(vcu[j, c, pl.ds(a, b - a), :], BF16)
                     for c in range(nc)], axis=1)

            if split_last and d == nc * 6 - 1:
                m = jnp.concatenate(
                    [_dot(lhs_of(*t0), rhs), _dot(lhs_of(*t1), rhs)], axis=0)
            elif nr == nb:
                m = _dot(lhs_of(0, nb), rhs)
            else:
                m = _dot(jnp.concatenate([lhs_of(*t0), lhs_of(*t1)], axis=0), rhs)
            ms.append(m)
            for r, t in sched.get(d, []):
                t(pltpu.bitcast(m[r * 8:(r + 1) * 8, :], U32) & zero)
            d += 1
        sink(n, ms)


def _k_region(v_cur, gw, ma, zero, nc, items, plan, pre):
    nb = NB0
    vcu = v_cur.bitcast(U32)
    gwu = gw.bitcast(U32)
    sched = _make_sched(plan, 2 * min(it[2] for it in items) // 8)
    ndots = nc * 6 * len(items)
    d = 0
    for k, (gi, b0, nr) in enumerate(items):
        cs = KG[gi]
        first = gi == 0
        rh = pl.ds(cs[0] * 64, len(cs) * 64)
        for t in pre[k]:
            t()
        order = ([(j, n) for j in JO for n in range(nc)] if first
                 else [(j, n) for n in range(nc) for j in JO])
        t0 = (b0, b0 + nr)
        t1 = (nb + b0, nb + b0 + nr)
        for j, n in order:
            rhs = pltpu.bitcast(gwu[j, n, rh, :], BF16)

            def lhs_of(a, b, j=j, cs=cs):
                return jnp.concatenate(
                    [pltpu.bitcast(vcu[j, c, pl.ds(a // 2, (b - a) // 2), :], BF16)
                     for c in cs], axis=1)

            def fin(m, ranges, j=j, n=n, first=first):
                off = 0
                outs = []
                for a, b in ranges:
                    mm = m[off:off + (b - a)]
                    if not first:
                        mm = mm + ma[n, j, pl.ds(a, b - a), :]
                    ma[n, j, pl.ds(a, b - a), :] = mm
                    outs.append(mm)
                    off += b - a
                return outs[0] if len(outs) == 1 else jnp.concatenate(outs, axis=0)

            if d >= ndots - 2:
                m = jnp.concatenate([fin(_dot(lhs_of(*t0), rhs), [t0]),
                                     fin(_dot(lhs_of(*t1), rhs), [t1])], axis=0)
            elif nr == nb:
                m = fin(_dot(lhs_of(0, 2 * nb), rhs), [(0, 2 * nb)])
            else:
                m = fin(_dot(jnp.concatenate([lhs_of(*t0), lhs_of(*t1)], axis=0), rhs),
                        [t0, t1])
            for r, t in sched.get(d, []):
                t(pltpu.bitcast(m[r * 8:(r + 1) * 8, :], U32) & zero)
            d += 1


def _kernel(x3_hbm, x_hbm, w_hbm, mean_hbm, var_hbm, g_hbm, b_hbm, o_hbm,
            xk, st, xall, oall, o0, va, vb, ma, gw, wl, pm, pv, pg, pb, ss, sems):
    C = w_hbm.shape[-1]
    B = x3_hbm.shape[0]
    nc = C // 128
    rpb = S * nc
    hr = rpb // 2
    pbs = SB * NSUB
    nq = (B - NB0 - SB) // pbs
    rqn = NB0 // nq
    q = pl.program_id(0)
    zero = jnp.full((8, 128), jax.lax.shift_right_logical(q, 24), jnp.int32).astype(U32)
    last_sem = 2 * (len(KG) - 1)
    osem = sems.at[1]
    xu_all = xall.bitcast(U32)
    ou_all = oall.bitcast(U32)

    def cp_in(b0, nb, sem):
        sl = pl.ds(b0 * rpb, nb * rpb)
        return pltpu.make_async_copy(x_hbm.at[sl, :], xall.at[sl, :], sem)

    def cp_out(src, b0, nb):
        sl = pl.ds(b0 * rpb, nb * rpb)
        return pltpu.make_async_copy(src.at[sl, :], o_hbm.at[sl, :], osem)

    def xk_copy(gi):
        sl = pl.ds(KG[gi][0] * S, len(KG[gi]) * S)
        return pltpu.make_async_copy(x3_hbm.at[pl.ds(0, NB0), sl, :], xk.at[:, sl, :],
                                     sems.at[min(2 * gi, last_sem)])

    def wk_copy(gi):
        sl = pl.ds(KG[gi][0] * 128, len(KG[gi]) * 128)
        return pltpu.make_async_copy(w_hbm.at[:, sl, :], wl.at[:, sl, :],
                                     sems.at[min(2 * gi + 1, last_sem)])

    def x1_copy():
        return cp_in(NB0, SB, sems.at[last_sem])

    def xq_copy(k):
        return cp_in(pl.multiple_of(NB0 + SB + k * pbs, 16), pbs, sems.at[0])

    def p_copies():
        return [pltpu.make_async_copy(s, d, sems.at[last_sem])
                for s, d in ((mean_hbm, pm), (var_hbm, pv), (g_hbm, pg), (b_hbm, pb))]

    def t_tasks(xu, v_ref, b0):
        return [functools.partial(_t_group, xu, v_ref, c, b0, rb, SB, nc)
                for c in range(nc) for rb in range(SB // RB)]

    def t0_tasks(gi, b0, nr):
        return [functools.partial(_t0_group, xk, st, va, c, rb, NB0)
                for rb in range(b0 // RB, (b0 + nr) // RB) for c in KG[gi]]

    def wt_thunks(gi):
        cs = KG[gi]
        return [functools.partial(_wt_piece, gw, wl, n, r0)
                for n in range(nc) for r0 in range(cs[0] * 128, (cs[-1] + 1) * 128, WR)]

    @pl.when(q == 0)
    def _startup():
        for gi in range(len(KG)):
            xk_copy(gi).start(priority=min(gi, 1))
            wk_copy(gi).start(priority=min(gi, 1))
        x1_copy().start(priority=1)
        for cp in p_copies():
            cp.start(priority=1)
        xk_copy(0).wait()
        for t in t0_tasks(0, 0, NB0):
            t()
        wt_done = set()
        t0_done = {0: NB0}
        for ri, reg in enumerate(R0P):
            last = ri == len(R0P) - 1
            gw_i = reg["wait"]
            if gw_i > 0:
                xk_copy(gw_i).wait()
            if reg.get("t0pre"):
                for t in t0_tasks(gw_i, 0, reg["t0pre"]):
                    t()
                t0_done[gw_i] = reg["t0pre"]
            wk_copy(gw_i).wait()
            if ri == 1:
                xq_copy(0).start(priority=1)
            if last:
                x1_copy().wait()
                for cp in p_copies():
                    cp.wait()
                mean = pm[...].astype(F32).reshape(1, C)
                var = pv[...].astype(F32).reshape(1, C)
                g = pg[...].astype(F32).reshape(1, C)
                b = pb[...].astype(F32).reshape(1, C)
                scf = g * jax.lax.rsqrt(var + 1e-5)
                sc = scf * 0.5
                ss[0:1, :] = sc
                ss[1:2, :] = (b - mean * scf) * 0.5
                for k, cst in enumerate((PA, PB_, A2, B2, A3, B3)):
                    ss[2 + k:3 + k, :] = sc * cst
            items = reg["items"]
            pre = []
            plan = []
            for k, (gi, b0, nr) in enumerate(items):
                th = []
                done = t0_done.get(gi, 0)
                if done < b0 + nr:
                    assert k > 0
                    plan.append((t0_tasks(gi, done, b0 + nr - done),
                                 [(k - 1) * 6 * nc + d for d in T0D]))
                    t0_done[gi] = b0 + nr
                if gi not in wt_done:
                    wt_done.add(gi)
                    th = wt_thunks(gi)
                pre.append(th)
            for gi, upto, dots in reg.get("t0x", ()):
                done = t0_done[gi]
                plan.append((t0_tasks(gi, done, upto - done), list(dots)))
                t0_done[gi] = upto
            if last:
                plan.append((t_tasks(xu_all, vb, NB0), list(TD)))
            _k_region(va, gw, ma, zero, nc, items, plan, pre)

    xq_copy(q).wait()
    for k in range(nq - 1):
        @pl.when(q == k + 1)
        def _(k=k):
            cp_out(o0, k * rqn, rqn).start()

    @pl.when(q < nq - 1)
    def _():
        xq_copy(q + 1).start()

    base = pl.multiple_of(NB0 + q * pbs, 16)
    xu = xu_all.at[pl.ds(pl.multiple_of(base * hr, 8), (pbs + SB) * hr), :]
    ou = ou_all.at[pl.ds(pl.multiple_of(base * hr, 8), pbs * hr), :]
    rq = pl.multiple_of(q * rqn, EB)
    ou0 = o0.bitcast(U32).at[pl.ds(pl.multiple_of(rq * hr, 8), rqn * hr), :]
    vbufs = (vb, va)
    e0 = [functools.partial(_epi_deferred, ma, ou0, ss, n, t, rq, r0, nc)
          for n in range(nc) for t in range(2) for r0 in range(0, rqn, EB)]
    for k in range(NSUB):
        ek = e0[(k * len(e0)) // NSUB:((k + 1) * len(e0)) // NSUB]
        _mm_region(vbufs[k % 2], gw, zero, nc, SB,
                   [(t_tasks(xu, vbufs[(k + 1) % 2], (k + 1) * SB), GDOTS), (ek, EDOTS)],
                   lambda n, ms, k=k: _epilogue(ms, ou, ss, n, k * SB, SB, nc),
                   k == NSUB - 1)
        cp_out(oall, base + k * SB, SB).start()

    @pl.when(q == nq - 1)
    def _finish():
        bl = B - SB
        cp_out(o0, (nq - 1) * rqn, rqn).start()
        pos = 0
        for k, nr in enumerate(LAST):
            _mm_region(vb, gw, zero, nc, SB, [],
                       lambda n, ms, pos=pos, nr=nr: _epilogue(
                           ms, ou_all, ss, n, bl + pos, nr, nc),
                       k == len(LAST) - 1, r0=pos, nr=nr)
            cp_out(oall, bl + pos, nr).start()
            pos += nr
        pltpu.make_async_copy(oall, o_hbm, osem).wait()


@jax.jit
def pallas_standalone__batchnorm__sampling_kernel(
    x: jax.Array,
    w: jax.Array,
    mean: jax.Array,
    var: jax.Array,
    g: jax.Array,
    b: jax.Array,
):
    B, seq, C = x.shape
    nc = C // 128
    nq = (B - NB0 - SB) // (SB * NSUB)
    assert seq == S and w.shape == (3, C, C) and nc == 5
    assert NB0 + nq * SB * NSUB + SB == B and sum(LAST) == SB
    assert NB0 % (nq * EB) == 0 and NSUB % 2 == 0
    x4 = x.reshape(B, S, nc, 128).transpose(0, 2, 1, 3)
    x2 = x4.reshape(B * nc * S, 128)
    x3 = x4.reshape(B, nc * S, 128)
    hbm = pl.BlockSpec(memory_space=pl.ANY)
    out = pl.pallas_call(
        _kernel,
        grid=(nq,),
        in_specs=[hbm] * 7,
        out_specs=hbm,
        out_shape=jax.ShapeDtypeStruct((B * S * nc, 128), x.dtype),
        scratch_shapes=[
            pltpu.VMEM((NB0, S * nc, 128), BF16),
            pltpu.VMEM((NB0 * S * nc // 2, 128), U32),
            pltpu.VMEM((B * S * nc, 128), BF16),
            pltpu.VMEM((B * S * nc, 128), BF16),
            pltpu.VMEM((NB0 * S * nc, 128), BF16),
            pltpu.VMEM((6, nc, 2 * NB0, 128), BF16),
            pltpu.VMEM((6, nc, 2 * NB0, 128), BF16),
            pltpu.VMEM((nc, 6, 2 * NB0, 128), F32),
            pltpu.VMEM((6, nc, C, 128), BF16),
            pltpu.VMEM((3, C, C), BF16),
            pltpu.VMEM((C,), BF16), pltpu.VMEM((C,), BF16),
            pltpu.VMEM((C,), BF16), pltpu.VMEM((C,), BF16),
            pltpu.VMEM((8, C), F32),
            pltpu.SemaphoreType.DMA((2 * len(KG) - 1,)),
        ],
        compiler_params=pltpu.CompilerParams(
            dimension_semantics=("arbitrary",),
            vmem_limit_bytes=100 * 1024 * 1024,
        ),
    )(x3, x2, w, mean, var, g, b)
    return out.reshape(B, nc, S, 128).transpose(0, 2, 1, 3).reshape(B, S, C)
```

```python
import functools

import jax
import jax.numpy as jnp
import jax.experimental.pallas as pl
import jax.experimental.pallas.tpu as pltpu

F32 = jnp.float32
BF16 = jnp.bfloat16
U32 = jnp.uint32

PA = 0.625
PB_ = 1.6
A2, B2 = PA * PA, PB_ * PB_
A3, B3 = A2 * PA, B2 * PB_
CC = A2 + B2
NA = 2 * A2 * (A2 - B2)
NB = 2 * B2 * (B2 - A2)

S = 8
RB = 16
EB = 8
WR = 32

NB0 = 192
SB = 64
NSUB = 4
LAST = (32, 16, 16)
KG = ((0,), (1, 2), (3, 4))
R0P = (
    dict(wait=0, items=((0, 0, 192),)),
    dict(wait=1, t0pre=96, items=((1, 0, 96), (1, 96, 64)),
         t0x=((1, 192, tuple(range(32, 56))),)),
    dict(wait=2, items=((1, 160, 32), (2, 0, 96), (2, 96, 96))),
)
JO = (0, 5, 1, 2, 3, 4)
GDOTS = tuple(d for d in range(27) if d % 6 in (1, 2))
EDOTS = (3, 9, 15, 21, 27)
TD = tuple(range(60, 88))
T0D = tuple(range(0, 26))


def _in_transform(d0, d1, d2, d3, d4, d5):
    t_b2 = B2 * d2
    t_a2 = A2 * d2
    e1 = d4 - t_b2
    e2 = d4 - t_a2
    o1 = PA * d3 - (PA * B2) * d1
    o2 = PB_ * d3 - (PB_ * A2) * d1
    v0 = e1 - t_a2
    if d0 is not None:
        v0 = v0 + d0
    v5 = d1 - CC * d3
    if d5 is not None:
        v5 = v5 + d5
    return [v0, e1 + o1, e1 - o1, e2 + o2, e2 - o2, v5]


def _rep(v, k):
    return v if k == 1 else jnp.concatenate([v] * k, axis=0)


def _t_store(xs, v_ref, c, rb, nb):
    v_t0 = _in_transform(None, xs[0], xs[1], xs[2], xs[3], xs[4])
    v_t1 = _in_transform(xs[3], xs[4], xs[5], xs[6], xs[7], None)
    for j in range(6):
        v_ref[j, c, pl.ds(rb * RB, RB), :] = v_t0[j].astype(BF16)
        v_ref[j, c, pl.ds(nb + rb * RB, RB), :] = v_t1[j].astype(BF16)


def _t_group(xu, v_ref, c, b0, rb, nb, nc, gate):
    sh = _rep(gate | jnp.uint32(16), RB // 8)
    mk = _rep(gate | jnp.uint32(0xFFFF0000), RB // 8)
    xs = []
    for p in range(4):
        wd = xu[pl.ds((b0 + rb * RB) * 4 * nc + c * 4 + p, RB, stride=4 * nc), :]
        xs.append(pltpu.bitcast(wd << sh, F32))
        xs.append(pltpu.bitcast(wd & mk, F32))
    _t_store(xs, v_ref, c, rb, nb)


def _t0_group(xk, cl, st, v_ref, c, rb, nb, gate=None):
    r0 = (c * (nb // RB) + rb) * RB * S // 2
    u = pltpu.bitcast(
        xk[pl.ds(rb * RB, RB), pl.ds(cl * S, S), :].reshape(RB * S, 128), U32)
    if gate is not None:
        u = u | _rep(gate, RB * S // 16)
    st[pl.ds(r0, RB * S // 2), :] = u
    xs = []
    for p in range(4):
        wd = st[pl.ds(r0 + p, RB, stride=4), :]
        xs.append(pltpu.bitcast(wd << 16, F32))
        xs.append(pltpu.bitcast(wd & jnp.uint32(0xFFFF0000), F32))
    _t_store(xs, v_ref, c, rb, nb)


def _wt_piece(gw, wl, rl, n, r0):
    rs = pl.ds(r0, WR)
    ns = pl.ds(n * 128, 128)
    gwu = gw.bitcast(U32)
    rh = pl.ds(r0 // 2, WR // 2)
    u0, u1, u2 = [pltpu.bitcast(wl[k, pl.ds(rl, WR), ns], U32) for k in range(3)]
    gwu[0, n, rh, :] = u0
    gwu[5, n, rh, :] = u2
    g0, g1, g2 = [pltpu.bitcast(u, BF16).astype(F32) for u in (u0, u1, u2)]
    ea = g0 * (1.0 / NA) + g2 * (A2 / NA)
    oa = g1 * (PA / NA)
    gw[1, n, rs, :] = (ea + oa).astype(BF16)
    gw[2, n, rs, :] = (ea - oa).astype(BF16)
    eb = g0 * (1.0 / NB) + g2 * (B2 / NB)
    ob = g1 * (PB_ / NB)
    gw[3, n, rs, :] = (eb + ob).astype(BF16)
    gw[4, n, rs, :] = (eb - ob).astype(BF16)


def _epilogue(ms, ou, ss, n, b0, nb, nc, tiles=(0, 1)):
    ns = slice(n * 128, (n + 1) * 128)
    cf = [ss[k:k + 1, ns] for k in range(8)]
    sc, sh = cf[0], cf[1]
    s1 = ms[1] + ms[2]
    d1 = ms[1] - ms[2]
    s2 = ms[3] + ms[4]
    d2 = ms[3] - ms[4]
    h = [
        (ms[0] + s1 + s2) * sc + sh,
        d1 * cf[2] + d2 * cf[3] + sh,
        s1 * cf[4] + s2 * cf[5] + sh,
        d1 * cf[6] + d2 * cf[7] + ms[5] * sc + sh,
    ]
    z = [hh + hh * jnp.tanh(hh) for hh in h]
    zr = [pltpu.bitcast(zz.astype(BF16).astype(F32), U32) for zz in z]
    p01 = (zr[0] >> 16) | zr[1]
    p23 = (zr[2] >> 16) | zr[3]
    base = b0 * 4 * nc + n * 4
    for k, t in enumerate(tiles):
        ou[pl.ds(base + 2 * t, nb, stride=4 * nc), :] = p01[k * nb:(k + 1) * nb]
        ou[pl.ds(base + 2 * t + 1, nb, stride=4 * nc), :] = p23[k * nb:(k + 1) * nb]


def _epi_deferred(m_ref, ou0, ss, n, t, rq, r0, nc, gate):
    ms = [m_ref[n, j, pl.ds(pl.multiple_of(rq + (t * NB0 + r0), 8), EB), :]
          for j in range(6)]
    gt = _rep(gate, EB // 8)
    for j in (0, 1, 3, 5):
        ms[j] = pltpu.bitcast(pltpu.bitcast(ms[j], U32) | gt, F32)
    _epilogue(ms, ou0, ss, n, r0, EB, nc, tiles=(t,))


def _make_sched(plan, nvr):
    sched = {}
    for tasks, dots in plan:
        total = len(dots) * nvr
        for k, t in enumerate(tasks):
            pos = (k * total) // len(tasks)
            sched.setdefault(dots[pos // nvr], []).append((pos % nvr, t))
    return sched


def _dot(lhs, rhs):
    return jnp.dot(lhs, rhs, preferred_element_type=F32)


def _mm_region(v_cur, gw, zero, nc, nb, plan, sink, split_last, r0=0, nr=None):
    nr = nb if nr is None else nr
    vcu = v_cur.bitcast(U32)
    gwu = gw.bitcast(U32)
    sched = _make_sched(plan, 2 * nr // 8)
    t0 = (r0 // 2, (r0 + nr) // 2)
    t1 = ((nb + r0) // 2, (nb + r0 + nr) // 2)
    d = 0
    for n in range(nc):
        ms = []
        for j in range(6):
            rhs = pltpu.bitcast(gwu[j, n], BF16)

            def lhs_of(a, b, j=j):
                return jnp.concatenate(
                    [pltpu.bitcast(vcu[j, c, pl.ds(a, b - a), :], BF16)
                     for c in range(nc)], axis=1)

            if split_last and d == nc * 6 - 1:
                m = jnp.concatenate(
                    [_dot(lhs_of(*t0), rhs), _dot(lhs_of(*t1), rhs)], axis=0)
            elif nr == nb:
                m = _dot(lhs_of(0, nb), rhs)
            else:
                m = _dot(jnp.concatenate([lhs_of(*t0), lhs_of(*t1)], axis=0), rhs)
            ms.append(m)
            for r, t in sched.get(d, []):
                t(pltpu.bitcast(m[r * 8:(r + 1) * 8, :], U32) & zero)
            d += 1
        sink(n, ms)


def _k_region(v_cur, gw, ma, zero, nc, items, plan, pre):
    nb = NB0
    vcu = v_cur.bitcast(U32)
    gwu = gw.bitcast(U32)
    sched = _make_sched(plan, 2 * min(it[2] for it in items) // 8)
    ndots = nc * 6 * len(items)
    d = 0
    for k, (gi, b0, nr) in enumerate(items):
        cs = KG[gi]
        first = gi == 0
        rh = pl.ds(cs[0] * 64, len(cs) * 64)
        for t in pre[k]:
            t()
        order = ([(j, n) for j in JO for n in range(nc)] if first
                 else [(j, n) for n in range(nc) for j in JO])
        t0 = (b0, b0 + nr)
        t1 = (nb + b0, nb + b0 + nr)
        for j, n in order:
            rhs = pltpu.bitcast(gwu[j, n, rh, :], BF16)

            def lhs_of(a, b, j=j, cs=cs):
                return jnp.concatenate(
                    [pltpu.bitcast(vcu[j, c, pl.ds(a // 2, (b - a) // 2), :], BF16)
                     for c in cs], axis=1)

            def fin(m, ranges, j=j, n=n, first=first):
                off = 0
                outs = []
                for a, b in ranges:
                    mm = m[off:off + (b - a)]
                    if not first:
                        mm = mm + ma[n, j, pl.ds(a, b - a), :]
                    ma[n, j, pl.ds(a, b - a), :] = mm
                    outs.append(mm)
                    off += b - a
                return outs[0] if len(outs) == 1 else jnp.concatenate(outs, axis=0)

            if d >= ndots - 2:
                m = jnp.concatenate([fin(_dot(lhs_of(*t0), rhs), [t0]),
                                     fin(_dot(lhs_of(*t1), rhs), [t1])], axis=0)
            elif nr == nb:
                m = fin(_dot(lhs_of(0, 2 * nb), rhs), [(0, 2 * nb)])
            else:
                m = fin(_dot(jnp.concatenate([lhs_of(*t0), lhs_of(*t1)], axis=0), rhs),
                        [t0, t1])
            for r, t in sched.get(d, []):
                t(pltpu.bitcast(m[r * 8:(r + 1) * 8, :], U32) & zero)
            d += 1


def _kernel(x3_hbm, x_hbm, w_hbm, mean_hbm, var_hbm, g_hbm, b_hbm, o_hbm,
            xk0, xk1, xk2, wl0, wl1, wl2, st, xall, oall, o0, va, vb, ma, gw,
            pm, pv, pg, pb, ss, sems):
    xks = (xk0, xk1, xk2)
    wls = (wl0, wl1, wl2)
    C = w_hbm.shape[-1]
    B = x3_hbm.shape[0]
    nc = C // 128
    rpb = S * nc
    hr = rpb // 2
    pbs = SB * NSUB
    nq = (B - NB0 - SB) // pbs
    rqn = NB0 // nq
    q = pl.program_id(0)
    zero = jnp.full((8, 128), jax.lax.shift_right_logical(q, 24), jnp.int32).astype(U32)
    last_sem = 2 * (len(KG) - 1)
    osem = sems.at[1]
    xu_all = xall.bitcast(U32)
    ou_all = oall.bitcast(U32)

    def cp_in(b0, nb, sem):
        sl = pl.ds(b0 * rpb, nb * rpb)
        return pltpu.make_async_copy(x_hbm.at[sl, :], xall.at[sl, :], sem)

    def cp_out(src, b0, nb):
        sl = pl.ds(b0 * rpb, nb * rpb)
        return pltpu.make_async_copy(src.at[sl, :], o_hbm.at[sl, :], osem)

    def xk_copy(gi):
        sl = pl.ds(KG[gi][0] * S, len(KG[gi]) * S)
        return pltpu.make_async_copy(x3_hbm.at[pl.ds(0, NB0), sl, :], xks[gi],
                                     sems.at[min(2 * gi, last_sem)])

    def wk_copy(gi):
        sl = pl.ds(KG[gi][0] * 128, len(KG[gi]) * 128)
        return pltpu.make_async_copy(w_hbm.at[:, sl, :], wls[gi],
                                     sems.at[min(2 * gi + 1, last_sem)])

    def x1_copy():
        return cp_in(NB0, SB, sems.at[last_sem])

    def xq_copy(k):
        return cp_in(pl.multiple_of(NB0 + SB + k * pbs, 16), pbs, sems.at[0])

    def p_copies():
        return [pltpu.make_async_copy(s, d, sems.at[last_sem])
                for s, d in ((mean_hbm, pm), (var_hbm, pv), (g_hbm, pg), (b_hbm, pb))]

    def t_tasks(xu, v_ref, b0):
        return [functools.partial(_t_group, xu, v_ref, c, b0, rb, SB, nc)
                for c in range(nc) for rb in range(SB // RB)]

    def t0_tasks(gi, b0, nr):
        return [functools.partial(_t0_group, xks[gi], c - KG[gi][0], st, va, c, rb, NB0)
                for rb in range(b0 // RB, (b0 + nr) // RB) for c in KG[gi]]

    def wt_thunks(gi):
        cs = KG[gi]
        return [functools.partial(_wt_piece, gw, wls[gi], r0 - cs[0] * 128, n, r0)
                for n in range(nc) for r0 in range(cs[0] * 128, (cs[-1] + 1) * 128, WR)]

    @pl.when(q == 0)
    def _startup():
        for gi in range(len(KG)):
            xk_copy(gi).start(priority=min(gi, 1))
            wk_copy(gi).start(priority=min(gi, 1))
        x1_copy().start(priority=1)
        for cp in p_copies():
            cp.start(priority=1)
        xk_copy(0).wait()
        for t in t0_tasks(0, 0, NB0):
            t()
        wt_done = set()
        t0_done = {0: NB0}
        for ri, reg in enumerate(R0P):
            last = ri == len(R0P) - 1
            gw_i = reg["wait"]
            if gw_i > 0:
                xk_copy(gw_i).wait()
            if reg.get("t0pre"):
                for t in t0_tasks(gw_i, 0, reg["t0pre"]):
                    t()
                t0_done[gw_i] = reg["t0pre"]
            wk_copy(gw_i).wait()
            if ri == 1:
                xq_copy(0).start(priority=1)
            if last:
                x1_copy().wait()
                for cp in p_copies():
                    cp.wait()
                mean = pm[...].astype(F32).reshape(1, C)
                var = pv[...].astype(F32).reshape(1, C)
                g = pg[...].astype(F32).reshape(1, C)
                b = pb[...].astype(F32).reshape(1, C)
                scf = g * jax.lax.rsqrt(var + 1e-5)
                sc = scf * 0.5
                ss[0:1, :] = sc
                ss[1:2, :] = (b - mean * scf) * 0.5
                for k, cst in enumerate((PA, PB_, A2, B2, A3, B3)):
                    ss[2 + k:3 + k, :] = sc * cst
            items = reg["items"]
            pre = []
            plan = []
            for k, (gi, b0, nr) in enumerate(items):
                th = []
                done = t0_done.get(gi, 0)
                if done < b0 + nr:
                    assert k > 0
                    plan.append((t0_tasks(gi, done, b0 + nr - done),
                                 [(k - 1) * 6 * nc + d for d in T0D]))
                    t0_done[gi] = b0 + nr
                if gi not in wt_done:
                    wt_done.add(gi)
                    th = wt_thunks(gi)
                pre.append(th)
            for gi, upto, dots in reg.get("t0x", ()):
                done = t0_done[gi]
                plan.append((t0_tasks(gi, done, upto - done), list(dots)))
                t0_done[gi] = upto
            if last:
                plan.append((t_tasks(xu_all, vb, NB0), list(TD)))
            _k_region(va, gw, ma, zero, nc, items, plan, pre)

    xq_copy(q).wait()
    for k in range(nq - 1):
        @pl.when(q == k + 1)
        def _(k=k):
            cp_out(o0, k * rqn, rqn).start()

    @pl.when(q < nq - 1)
    def _():
        xq_copy(q + 1).start()

    base = pl.multiple_of(NB0 + q * pbs, 16)
    xu = xu_all.at[pl.ds(pl.multiple_of(base * hr, 8), (pbs + SB) * hr), :]
    ou = ou_all.at[pl.ds(pl.multiple_of(base * hr, 8), pbs * hr), :]
    rq = pl.multiple_of(q * rqn, EB)
    ou0 = o0.bitcast(U32).at[pl.ds(pl.multiple_of(rq * hr, 8), rqn * hr), :]
    vbufs = (vb, va)
    e0 = [functools.partial(_epi_deferred, ma, ou0, ss, n, t, rq, r0, nc)
          for n in range(nc) for t in range(2) for r0 in range(0, rqn, EB)]
    for k in range(NSUB):
        ek = e0[(k * len(e0)) // NSUB:((k + 1) * len(e0)) // NSUB]
        _mm_region(vbufs[k % 2], gw, zero, nc, SB,
                   [(t_tasks(xu, vbufs[(k + 1) % 2], (k + 1) * SB), GDOTS), (ek, EDOTS)],
                   lambda n, ms, k=k: _epilogue(ms, ou, ss, n, k * SB, SB, nc),
                   k == NSUB - 1)
        cp_out(oall, base + k * SB, SB).start()

    @pl.when(q == nq - 1)
    def _finish():
        bl = B - SB
        cp_out(o0, (nq - 1) * rqn, rqn).start()
        pos = 0
        for k, nr in enumerate(LAST):
            _mm_region(vb, gw, zero, nc, SB, [],
                       lambda n, ms, pos=pos, nr=nr: _epilogue(
                           ms, ou_all, ss, n, bl + pos, nr, nc),
                       k == len(LAST) - 1, r0=pos, nr=nr)
            cp_out(oall, bl + pos, nr).start()
            pos += nr
        pltpu.make_async_copy(oall, o_hbm, osem).wait()


@jax.jit
def pallas_standalone__batchnorm__sampling_kernel(
    x: jax.Array,
    w: jax.Array,
    mean: jax.Array,
    var: jax.Array,
    g: jax.Array,
    b: jax.Array,
):
    B, seq, C = x.shape
    nc = C // 128
    nq = (B - NB0 - SB) // (SB * NSUB)
    assert seq == S and w.shape == (3, C, C) and nc == 5
    assert NB0 + nq * SB * NSUB + SB == B and sum(LAST) == SB
    assert NB0 % (nq * EB) == 0 and NSUB % 2 == 0
    x4 = x.reshape(B, S, nc, 128).transpose(0, 2, 1, 3)
    x2 = x4.reshape(B * nc * S, 128)
    x3 = x4.reshape(B, nc * S, 128)
    hbm = pl.BlockSpec(memory_space=pl.ANY)
    out = pl.pallas_call(
        _kernel,
        grid=(nq,),
        in_specs=[hbm] * 7,
        out_specs=hbm,
        out_shape=jax.ShapeDtypeStruct((B * S * nc, 128), x.dtype),
        scratch_shapes=[
            *[pltpu.VMEM((NB0, S * len(cs), 128), BF16) for cs in KG],
            *[pltpu.VMEM((3, 128 * len(cs), C), BF16) for cs in KG],
            pltpu.VMEM((NB0 * S * nc // 2, 128), U32),
            pltpu.VMEM((B * S * nc, 128), BF16),
            pltpu.VMEM((B * S * nc, 128), BF16),
            pltpu.VMEM((NB0 * S * nc, 128), BF16),
            pltpu.VMEM((6, nc, 2 * NB0, 128), BF16),
            pltpu.VMEM((6, nc, 2 * NB0, 128), BF16),
            pltpu.VMEM((nc, 6, 2 * NB0, 128), F32),
            pltpu.VMEM((6, nc, C, 128), BF16),
            pltpu.VMEM((C,), BF16), pltpu.VMEM((C,), BF16),
            pltpu.VMEM((C,), BF16), pltpu.VMEM((C,), BF16),
            pltpu.VMEM((8, C), F32),
            pltpu.SemaphoreType.DMA((2 * len(KG) - 1,)),
        ],
        compiler_params=pltpu.CompilerParams(
            dimension_semantics=("arbitrary",),
            vmem_limit_bytes=100 * 1024 * 1024,
        ),
    )(x3, x2, w, mean, var, g, b)
    return out.reshape(B, nc, S, 128).transpose(0, 2, 1, 3).reshape(B, S, C)
```

```python
import functools

import jax
import jax.numpy as jnp
import jax.experimental.pallas as pl
import jax.experimental.pallas.tpu as pltpu

F32 = jnp.float32
BF16 = jnp.bfloat16
U32 = jnp.uint32

PA = 0.625
PB_ = 1.6
A2, B2 = PA * PA, PB_ * PB_
A3, B3 = A2 * PA, B2 * PB_
CC = A2 + B2
NA = 2 * A2 * (A2 - B2)
NB = 2 * B2 * (B2 - A2)

S = 8
RB = 16
EB = 8
WR = 32
PAD = 64

NB0 = 192
SB = 64
NSUB = 4
LAST = (32, 16, 16)
KG = ((0,), (1, 2), (3, 4))
R0P = (
    dict(wait=0, items=((0, 0, 192),)),
    dict(wait=1, t0pre=96, items=((1, 0, 96), (1, 96, 64)),
         t0x=((1, 192, tuple(range(32, 56))),)),
    dict(wait=2, items=((1, 160, 32), (2, 0, 96), (2, 96, 96))),
)
JO = (0, 5, 1, 2, 3, 4)
GDOTS = tuple(d for d in range(27) if d % 6 in (1, 2))
EDOTS = (3, 9, 15, 21, 27)
TD = tuple(range(60, 88))
T0D = tuple(range(0, 26))


def _in_transform(d0, d1, d2, d3, d4, d5):
    t_b2 = B2 * d2
    t_a2 = A2 * d2
    e1 = d4 - t_b2
    e2 = d4 - t_a2
    o1 = PA * d3 - (PA * B2) * d1
    o2 = PB_ * d3 - (PB_ * A2) * d1
    v0 = e1 - t_a2
    if d0 is not None:
        v0 = v0 + d0
    v5 = d1 - CC * d3
    if d5 is not None:
        v5 = v5 + d5
    return [v0, e1 + o1, e1 - o1, e2 + o2, e2 - o2, v5]


def _rep(v, k):
    return v if k == 1 else jnp.concatenate([v] * k, axis=0)


def _t_store(xs, v_ref, c, rb, nb):
    v_t0 = _in_transform(None, xs[0], xs[1], xs[2], xs[3], xs[4])
    v_t1 = _in_transform(xs[3], xs[4], xs[5], xs[6], xs[7], None)
    for j in range(6):
        v_ref[j, c, pl.ds(rb * RB, RB), :] = v_t0[j].astype(BF16)
        v_ref[j, c, pl.ds(nb + rb * RB, RB), :] = v_t1[j].astype(BF16)


def _t_group(xu, v_ref, c, b0, rb, nb, nc, gate):
    sh = _rep(gate | jnp.uint32(16), RB // 8)
    mk = _rep(gate | jnp.uint32(0xFFFF0000), RB // 8)
    xs = []
    for p in range(4):
        wd = xu[pl.ds((b0 + rb * RB) * 4 * nc + c * 4 + p, RB, stride=4 * nc), :]
        xs.append(pltpu.bitcast(wd << sh, F32))
        xs.append(pltpu.bitcast(wd & mk, F32))
    _t_store(xs, v_ref, c, rb, nb)


def _t0_group(xk, cl, st, v_ref, c, rb, nb, gate=None):
    r0 = (c * (nb // RB) + rb) * RB * S // 2
    u = pltpu.bitcast(
        xk[pl.ds(rb * RB, RB), pl.ds(cl * S, S), :].reshape(RB * S, 128), U32)
    if gate is not None:
        u = u | _rep(gate, RB * S // 16)
    st[pl.ds(r0, RB * S // 2), :] = u
    xs = []
    for p in range(4):
        wd = st[pl.ds(r0 + p, RB, stride=4), :]
        xs.append(pltpu.bitcast(wd << 16, F32))
        xs.append(pltpu.bitcast(wd & jnp.uint32(0xFFFF0000), F32))
    _t_store(xs, v_ref, c, rb, nb)


def _wt_piece(gw, wl, rl, n, r0):
    rs = pl.ds(r0, WR)
    ns = pl.ds(n * 128, 128)
    gwu = gw.bitcast(U32)
    rh = pl.ds(r0 // 2, WR // 2)
    u0, u1, u2 = [pltpu.bitcast(wl[k, pl.ds(rl, WR), ns], U32) for k in range(3)]
    gwu[0, n, rh, :] = u0
    gwu[5, n, rh, :] = u2
    g0, g1, g2 = [pltpu.bitcast(u, BF16).astype(F32) for u in (u0, u1, u2)]
    ea = g0 * (1.0 / NA) + g2 * (A2 / NA)
    oa = g1 * (PA / NA)
    gw[1, n, rs, :] = (ea + oa).astype(BF16)
    gw[2, n, rs, :] = (ea - oa).astype(BF16)
    eb = g0 * (1.0 / NB) + g2 * (B2 / NB)
    ob = g1 * (PB_ / NB)
    gw[3, n, rs, :] = (eb + ob).astype(BF16)
    gw[4, n, rs, :] = (eb - ob).astype(BF16)


def _epilogue(ms, ou, ss, n, b0, nb, nc, tiles=(0, 1)):
    ns = slice(n * 128, (n + 1) * 128)
    cf = [ss[k:k + 1, ns] for k in range(8)]
    sc, sh = cf[0], cf[1]
    s1 = ms[1] + ms[2]
    d1 = ms[1] - ms[2]
    s2 = ms[3] + ms[4]
    d2 = ms[3] - ms[4]
    h = [
        (ms[0] + s1 + s2) * sc + sh,
        d1 * cf[2] + d2 * cf[3] + sh,
        s1 * cf[4] + s2 * cf[5] + sh,
        d1 * cf[6] + d2 * cf[7] + ms[5] * sc + sh,
    ]
    z = [hh + hh * jnp.tanh(hh) for hh in h]
    zr = [pltpu.bitcast(zz.astype(BF16).astype(F32), U32) for zz in z]
    p01 = (zr[0] >> 16) | zr[1]
    p23 = (zr[2] >> 16) | zr[3]
    base = b0 * 4 * nc + n * 4
    for k, t in enumerate(tiles):
        ou[pl.ds(base + 2 * t, nb, stride=4 * nc), :] = p01[k * nb:(k + 1) * nb]
        ou[pl.ds(base + 2 * t + 1, nb, stride=4 * nc), :] = p23[k * nb:(k + 1) * nb]


def _epi_deferred(m_ref, ou0, ss, n, t, rq, r0, nc, gate):
    ms = [m_ref[n, j, pl.ds(pl.multiple_of(rq + (t * NB0 + r0), 8), EB), :]
          for j in range(6)]
    gt = _rep(gate, EB // 8)
    for j in (0, 1, 3, 5):
        ms[j] = pltpu.bitcast(pltpu.bitcast(ms[j], U32) | gt, F32)
    _epilogue(ms, ou0, ss, n, r0, EB, nc, tiles=(t,))


def _make_sched(plan, nvr):
    sched = {}
    for tasks, dots in plan:
        total = len(dots) * nvr
        for k, t in enumerate(tasks):
            pos = (k * total) // len(tasks)
            sched.setdefault(dots[pos // nvr], []).append((pos % nvr, t))
    return sched


def _dot(lhs, rhs):
    return jnp.dot(lhs, rhs, preferred_element_type=F32)


def _mm_region(v_cur, gw, zero, nc, nb, plan, sink, split_last, r0=0, nr=None):
    nr = nb if nr is None else nr
    vcu = v_cur.bitcast(U32)
    gwu = gw.bitcast(U32)
    sched = _make_sched(plan, 2 * nr // 8)
    t0 = (r0 // 2, (r0 + nr) // 2)
    t1 = ((nb + r0) // 2, (nb + r0 + nr) // 2)
    d = 0
    for n in range(nc):
        ms = []
        for j in range(6):
            rhs = pltpu.bitcast(gwu[j, n], BF16)

            def lhs_of(a, b, j=j):
                return jnp.concatenate(
                    [pltpu.bitcast(vcu[j, c, pl.ds(a, b - a), :], BF16)
                     for c in range(nc)], axis=1)

            if split_last and d == nc * 6 - 1:
                m = jnp.concatenate(
                    [_dot(lhs_of(*t0), rhs), _dot(lhs_of(*t1), rhs)], axis=0)
            elif nr == nb:
                m = _dot(lhs_of(0, nb), rhs)
            else:
                m = _dot(jnp.concatenate([lhs_of(*t0), lhs_of(*t1)], axis=0), rhs)
            ms.append(m)
            for r, t in sched.get(d, []):
                t(pltpu.bitcast(m[r * 8:(r + 1) * 8, :], U32) & zero)
            d += 1
        sink(n, ms)


def _k_region(v_cur, gw, ma, zero, nc, items, plan, pre):
    nb = NB0
    vcu = v_cur.bitcast(U32)
    gwu = gw.bitcast(U32)
    sched = _make_sched(plan, 2 * min(it[2] for it in items) // 8)
    ndots = nc * 6 * len(items)
    d = 0
    for k, (gi, b0, nr) in enumerate(items):
        cs = KG[gi]
        first = gi == 0
        rh = pl.ds(cs[0] * 64, len(cs) * 64)
        for t in pre[k]:
            t()
        order = ([(j, n) for j in JO for n in range(nc)] if first
                 else [(j, n) for n in range(nc) for j in JO])
        t0 = (b0, b0 + nr)
        t1 = (nb + b0, nb + b0 + nr)
        for j, n in order:
            rhs = pltpu.bitcast(gwu[j, n, rh, :], BF16)

            def lhs_of(a, b, j=j, cs=cs):
                return jnp.concatenate(
                    [pltpu.bitcast(vcu[j, c, pl.ds(a // 2, (b - a) // 2), :], BF16)
                     for c in cs], axis=1)

            def fin(m, ranges, j=j, n=n, first=first):
                off = 0
                outs = []
                for a, b in ranges:
                    mm = m[off:off + (b - a)]
                    if not first:
                        mm = mm + ma[n, j, pl.ds(a, b - a), :]
                    ma[n, j, pl.ds(a, b - a), :] = mm
                    outs.append(mm)
                    off += b - a
                return outs[0] if len(outs) == 1 else jnp.concatenate(outs, axis=0)

            if d >= ndots - 2:
                m = jnp.concatenate([fin(_dot(lhs_of(*t0), rhs), [t0]),
                                     fin(_dot(lhs_of(*t1), rhs), [t1])], axis=0)
            elif nr == nb:
                m = fin(_dot(lhs_of(0, 2 * nb), rhs), [(0, 2 * nb)])
            else:
                m = fin(_dot(jnp.concatenate([lhs_of(*t0), lhs_of(*t1)], axis=0), rhs),
                        [t0, t1])
            for r, t in sched.get(d, []):
                t(pltpu.bitcast(m[r * 8:(r + 1) * 8, :], U32) & zero)
            d += 1


def _kernel(x3_hbm, x_hbm, w_hbm, mean_hbm, var_hbm, g_hbm, b_hbm, o_hbm,
            xk0, xk1, xk2, wl0, wl1, wl2, st, x1b, xqb, oall, o0, va, vb, ma, gw,
            pm, pv, pg, pb, ss, sems):
    xks = (xk0, xk1, xk2)
    wls = (wl0, wl1, wl2)
    C = w_hbm.shape[-1]
    B = x3_hbm.shape[0]
    nc = C // 128
    rpb = S * nc
    hr = rpb // 2
    pbs = SB * NSUB
    nq = (B - NB0 - SB) // pbs
    rqn = NB0 // nq
    q = pl.program_id(0)
    zero = jnp.full((8, 128), jax.lax.shift_right_logical(q, 24), jnp.int32).astype(U32)
    last_sem = 2 * (len(KG) - 1)
    osem = sems.at[1]
    ou_all = oall.bitcast(U32)

    def cp_out(src, b0, nb):
        sl = pl.ds(b0 * rpb, nb * rpb)
        return pltpu.make_async_copy(src.at[sl, :], o_hbm.at[sl, :], osem)

    def xk_copy(gi):
        sl = pl.ds(KG[gi][0] * S, len(KG[gi]) * S)
        return pltpu.make_async_copy(x3_hbm.at[pl.ds(0, NB0), sl, :], xks[gi],
                                     sems.at[min(2 * gi, last_sem)])

    def wk_copy(gi):
        sl = pl.ds(KG[gi][0] * 128, len(KG[gi]) * 128)
        return pltpu.make_async_copy(w_hbm.at[:, sl, :], wls[gi],
                                     sems.at[min(2 * gi + 1, last_sem)])

    def x1_copy():
        return pltpu.make_async_copy(x_hbm.at[pl.ds(NB0 * rpb, SB * rpb), :],
                                     x1b.at[pl.ds(0, SB * rpb), :], sems.at[last_sem])

    def xq_copy(k):
        r0 = pl.multiple_of((NB0 + SB + k * pbs) * rpb, 16)
        return pltpu.make_async_copy(x_hbm.at[pl.ds(r0, pbs * rpb), :],
                                     xqb.at[k, pl.ds(0, pbs * rpb), :], sems.at[0])

    def p_copies():
        return [pltpu.make_async_copy(s, d, sems.at[last_sem])
                for s, d in ((mean_hbm, pm), (var_hbm, pv), (g_hbm, pg), (b_hbm, pb))]

    def t_tasks(xu, v_ref, b0):
        return [functools.partial(_t_group, xu, v_ref, c, b0, rb, SB, nc)
                for c in range(nc) for rb in range(SB // RB)]

    def t0_tasks(gi, b0, nr):
        return [functools.partial(_t0_group, xks[gi], c - KG[gi][0], st, va, c, rb, NB0)
                for rb in range(b0 // RB, (b0 + nr) // RB) for c in KG[gi]]

    def wt_thunks(gi):
        cs = KG[gi]
        return [functools.partial(_wt_piece, gw, wls[gi], r0 - cs[0] * 128, n, r0)
                for n in range(nc) for r0 in range(cs[0] * 128, (cs[-1] + 1) * 128, WR)]

    @pl.when(q == 0)
    def _startup():
        for gi in range(len(KG)):
            xk_copy(gi).start(priority=min(gi, 1))
            wk_copy(gi).start(priority=min(gi, 1))
        x1_copy().start(priority=1)
        for cp in p_copies():
            cp.start(priority=1)
        xk_copy(0).wait()
        for t in t0_tasks(0, 0, NB0):
            t()
        wt_done = set()
        t0_done = {0: NB0}
        for ri, reg in enumerate(R0P):
            last = ri == len(R0P) - 1
            gw_i = reg["wait"]
            if gw_i > 0:
                xk_copy(gw_i).wait()
            if reg.get("t0pre"):
                for t in t0_tasks(gw_i, 0, reg["t0pre"]):
                    t()
                t0_done[gw_i] = reg["t0pre"]
            wk_copy(gw_i).wait()
            if ri == 1:
                xq_copy(0).start(priority=1)
            if last:
                x1_copy().wait()
                for cp in p_copies():
                    cp.wait()
                mean = pm[...].astype(F32).reshape(1, C)
                var = pv[...].astype(F32).reshape(1, C)
                g = pg[...].astype(F32).reshape(1, C)
                b = pb[...].astype(F32).reshape(1, C)
                scf = g * jax.lax.rsqrt(var + 1e-5)
                sc = scf * 0.5
                ss[0:1, :] = sc
                ss[1:2, :] = (b - mean * scf) * 0.5
                for k, cst in enumerate((PA, PB_, A2, B2, A3, B3)):
                    ss[2 + k:3 + k, :] = sc * cst
            items = reg["items"]
            pre = []
            plan = []
            for k, (gi, b0, nr) in enumerate(items):
                th = []
                done = t0_done.get(gi, 0)
                if done < b0 + nr:
                    assert k > 0
                    plan.append((t0_tasks(gi, done, b0 + nr - done),
                                 [(k - 1) * 6 * nc + d for d in T0D]))
                    t0_done[gi] = b0 + nr
                if gi not in wt_done:
                    wt_done.add(gi)
                    th = wt_thunks(gi)
                pre.append(th)
            for gi, upto, dots in reg.get("t0x", ()):
                done = t0_done[gi]
                plan.append((t0_tasks(gi, done, upto - done), list(dots)))
                t0_done[gi] = upto
            if last:
                plan.append((t_tasks(x1b.bitcast(U32), vb, 0), list(TD)))
            _k_region(va, gw, ma, zero, nc, items, plan, pre)

    xq_copy(q).wait()
    for k in range(nq - 1):
        @pl.when(q == k + 1)
        def _(k=k):
            cp_out(o0, k * rqn, rqn).start()

    @pl.when(q < nq - 1)
    def _():
        xq_copy(q + 1).start()

    base = pl.multiple_of(NB0 + q * pbs, 16)
    xu = xqb.bitcast(U32).at[q]
    ou = ou_all.at[pl.ds(pl.multiple_of(base * hr, 8), pbs * hr + PAD // 2), :]
    rq = pl.multiple_of(q * rqn, EB)
    ou0 = o0.bitcast(U32).at[pl.ds(pl.multiple_of(rq * hr, 8), rqn * hr + PAD // 2), :]
    vbufs = (vb, va)
    e0 = [functools.partial(_epi_deferred, ma, ou0, ss, n, t, rq, r0, nc)
          for n in range(nc) for t in range(2) for r0 in range(0, rqn, EB)]
    for k in range(NSUB):
        ek = e0[(k * len(e0)) // NSUB:((k + 1) * len(e0)) // NSUB]
        _mm_region(vbufs[k % 2], gw, zero, nc, SB,
                   [(t_tasks(xu, vbufs[(k + 1) % 2], k * SB), GDOTS), (ek, EDOTS)],
                   lambda n, ms, k=k: _epilogue(ms, ou, ss, n, k * SB, SB, nc),
                   k == NSUB - 1)
        cp_out(oall, base + k * SB, SB).start()

    @pl.when(q == nq - 1)
    def _finish():
        bl = B - SB
        cp_out(o0, (nq - 1) * rqn, rqn).start()
        pos = 0
        for k, nr in enumerate(LAST):
            _mm_region(vb, gw, zero, nc, SB, [],
                       lambda n, ms, pos=pos, nr=nr: _epilogue(
                           ms, ou_all, ss, n, bl + pos, nr, nc),
                       k == len(LAST) - 1, r0=pos, nr=nr)
            cp_out(oall, bl + pos, nr).start()
            pos += nr
        pltpu.make_async_copy(o_hbm, o_hbm, osem).wait()


@jax.jit
def pallas_standalone__batchnorm__sampling_kernel(
    x: jax.Array,
    w: jax.Array,
    mean: jax.Array,
    var: jax.Array,
    g: jax.Array,
    b: jax.Array,
):
    B, seq, C = x.shape
    nc = C // 128
    nq = (B - NB0 - SB) // (SB * NSUB)
    assert seq == S and w.shape == (3, C, C) and nc == 5
    assert NB0 + nq * SB * NSUB + SB == B and sum(LAST) == SB
    assert NB0 % (nq * EB) == 0 and NSUB % 2 == 0
    x4 = x.reshape(B, S, nc, 128).transpose(0, 2, 1, 3)
    x2 = x4.reshape(B * nc * S, 128)
    x3 = x4.reshape(B, nc * S, 128)
    hbm = pl.BlockSpec(memory_space=pl.ANY)
    out = pl.pallas_call(
        _kernel,
        grid=(nq,),
        in_specs=[hbm] * 7,
        out_specs=hbm,
        out_shape=jax.ShapeDtypeStruct((B * S * nc, 128), x.dtype),
        scratch_shapes=[
            *[pltpu.VMEM((NB0, S * len(cs), 128), BF16) for cs in KG],
            *[pltpu.VMEM((3, 128 * len(cs), C), BF16) for cs in KG],
            pltpu.VMEM((NB0 * S * nc // 2 + PAD // 2, 128), U32),
            pltpu.VMEM((SB * S * nc + PAD, 128), BF16),
            pltpu.VMEM((nq, SB * NSUB * S * nc + PAD, 128), BF16),
            pltpu.VMEM((B * S * nc + PAD, 128), BF16),
            pltpu.VMEM((NB0 * S * nc + PAD, 128), BF16),
            pltpu.VMEM((6, nc, 2 * NB0, 128), BF16),
            pltpu.VMEM((6, nc, 2 * NB0, 128), BF16),
            pltpu.VMEM((nc, 6, 2 * NB0, 128), F32),
            pltpu.VMEM((6, nc, C, 128), BF16),
            pltpu.VMEM((C,), BF16), pltpu.VMEM((C,), BF16),
            pltpu.VMEM((C,), BF16), pltpu.VMEM((C,), BF16),
            pltpu.VMEM((8, C), F32),
            pltpu.SemaphoreType.DMA((2 * len(KG) - 1,)),
        ],
        compiler_params=pltpu.CompilerParams(
            dimension_semantics=("arbitrary",),
            vmem_limit_bytes=100 * 1024 * 1024,
        ),
    )(x3, x2, w, mean, var, g, b)
    return out.reshape(B, nc, S, 128).transpose(0, 2, 1, 3).reshape(B, S, C)
```
